```python
import os as _os
_os.environ.setdefault("JAX_PLATFORMS", "cpu")
import jax
import jax.numpy as jnp

def _softmax(x, axis=-1):
    return jax.nn.softmax(x, axis=axis)
def _gelu(x):
    return jax.nn.gelu(x, approximate=True)
def _silu(x):
    return jax.nn.silu(x)
def _sigmoid(x):
    return jax.nn.sigmoid(x)
def _layernorm(x, axis=-1, eps=1e-5):
    m = jnp.mean(x, axis=axis, keepdims=True)
    v = jnp.var(x, axis=axis, keepdims=True)
    return (x - m) / jnp.sqrt(v + eps)
def _scatter_add(tgt, idx, src, axis=0):
    return tgt.at[idx].add(src)
def _segment_sum(src, seg, n):
    return jax.ops.segment_sum(src, seg, n)
class _Rng:
    def __init__(self, key):
        self._k = key
    def _next(self):
        self._k, sub = jax.random.split(self._k)
        return sub
    def normal(self, shape):
        return jax.random.normal(self._next(), shape, dtype=jnp.bfloat16)
    def randint(self, lo, hi, shape):
        return jax.random.randint(self._next(), shape, lo, hi, dtype=jnp.int32)
    def uniform(self, shape, lo=0.0, hi=1.0):
        return jax.random.uniform(self._next(), shape, jnp.bfloat16, lo, hi)
    def permutation(self, n):
        return jax.random.permutation(self._next(), n)


kernel_name = 'parallel_sum__mha_block__swiglu_ffn__prompt'

def setup_inputs():
    _rng = _Rng(jax.random.key(int.from_bytes(__import__("os").urandom(4), "little")))
    _w = (lambda a: (lambda t: t.astype(jnp.bfloat16) if jnp.issubdtype(t.dtype, jnp.floating) else t)(jnp.asarray(a)))
    def _A_setup():
        B, S, D, H = 1, 2048, 512, 32
        return {
            "x": _w((lambda *s: _rng.normal(s) * 0.05)(B, S, D)),
            "wqkv": _w((lambda *s: _rng.normal(s) * 0.1)(D, 3 * D)),
            "wo": _w((lambda *s: _rng.normal(s) * 0.05)(D, D)),
        }
    _A_in = _A_setup()

    def _B_setup():
        B, S, D, F = 1, 2048, 512, 1792
        return {
            "x": _w((lambda *s: _rng.normal(s) * 0.05)(B, S, D)),
            "w_gate": _w((lambda *s: _rng.normal(s) * 0.05)(D, F)),
            "w_up": _w((lambda *s: _rng.normal(s) * 0.05)(D, F)),
            "w_down": _w((lambda *s: _rng.normal(s) * 0.05)(F, D)),
        }
    _B_in = _B_setup()

    return {
        "A_x": _A_in["x"],
        "A_wqkv": _A_in["wqkv"],
        "A_wo": _A_in["wo"],
        "B_x": _B_in["x"],
        "B_w_gate": _B_in["w_gate"],
        "B_w_up": _B_in["w_up"],
        "B_w_down": _B_in["w_down"],
    }

def reference(A_x, A_wqkv, A_wo, B_x, B_w_gate, B_w_up, B_w_down):
    def _A_ref(x, wqkv, wo):
        B, S, D = x.shape
        H = 32
        Dh = D // H
        qkv = (lambda x, *d: x.transpose(*d))((x @ wqkv).reshape(B, S, 3, H, Dh), 2, 0, 3, 1, 4)
        q, k, v = qkv[0], qkv[1], qkv[2]
        scores = jnp.einsum("bhqd,bhkd->bhqk", q, k) * (Dh ** -0.5)
        p = _softmax(scores, axis=-1)
        o = jnp.einsum("bhqk,bhkd->bhqd", p, v)
        return (lambda x, *d: x.transpose(*d))(o, 0, 2, 1, 3).reshape(B, S, D) @ wo

    def _B_ref(x, w_gate, w_up, w_down):
        g = _silu(x @ w_gate)
        u = x @ w_up
        return (g * u) @ w_down

    x = A_x
    xn = _layernorm(x, axis=-1)
    return x + _A_ref(xn, A_wqkv, A_wo) + _B_ref(xn, B_w_gate, B_w_up, B_w_down)
```

```python
import jax
import jax.numpy as jnp
import numpy as np
from jax import lax
import jax.experimental.pallas as pl
import jax.experimental.pallas.tpu as pltpu

S, D, H, DH, F = 2048, 512, 32, 16, 1792
f32, bf16 = jnp.float32, jnp.bfloat16
QSCALE = float(DH ** -0.5 * np.log2(np.e))
NT = (((1,), (1,)), ((), ()))
XC_ = 256


def make(bq=512, ck=128, U=2, dep=1, fi=1, rb=0, XC=256, order=0, c8=1, pv=0, seq=0, mseq=0, early=1, sd=-1, flags=None):
  nck = S // ck

  def kern(x_hbm, wqkv_hbm, wo_hbm, wg_hbm, wu_hbm, wd_hbm, o_ref,
           x_ref, wqkv_ref, wo_ref, wg_ref, wu_ref, wd_ref, sems,
           xn_ref, k_ref, vt_ref, wqt_ref, qt_ref, ot_ref, s_ref, a_ref, wvt_ref, ob_ref):
    i = pl.program_id(0)
    nx = S // XC

    def x_copy(c):
      r = pl.ds(c * XC, XC)
      return pltpu.make_async_copy(x_hbm.at[r, :], x_ref.at[r, :], sems.at[c])
    def w_copy(j):
      cols = pl.ds(j * D, D)
      return pltpu.make_async_copy(wqkv_hbm.at[:, cols], wqkv_ref.at[:, cols], sems.at[nx + j])
    late = [pltpu.make_async_copy(a, b, sems.at[nx + 3 + j]) for j, (a, b) in enumerate(
        ((wg_hbm, wg_ref), (wu_hbm, wu_ref), (wd_hbm, wd_ref), (wo_hbm, wo_ref)))]

    @pl.when(i == 0)
    def _():
      def ln(c):
        r = slice(c * XC, (c + 1) * XC)
        x = x_ref[r, :].astype(f32)
        xc = x - jnp.mean(x, axis=-1, keepdims=True)
        v = jnp.mean(xc * xc, axis=-1, keepdims=True)
        xn_ref[r, :] = (xc * lax.rsqrt(v + 1e-5)).astype(bf16)
      def proj(c):
        r = slice(c * XC, (c + 1) * XC)
        xn = xn_ref[r, :]
        kk = jnp.dot(xn, wqkv_ref[:, D:2 * D], preferred_element_type=f32).astype(bf16)
        for g in range(4):
          k_ref[g, r, :] = kk[:, g * 128:(g + 1) * 128]
        vt_ref[c] = lax.dot_general(wvt_ref[...], xn, NT, preferred_element_type=f32).astype(bf16).reshape(H, DH, XC)
      first = [x_copy(0), w_copy(1), w_copy(2)]
      second = [x_copy(c) for c in range(1, nx)] + [w_copy(0)]
      if pv == 0:
        for cp in first + second:
          cp.start()
      else:
        for cp in first:
          cp.start()
      qt_ref[...] = jnp.zeros(qt_ref.shape, bf16)
      first[0].wait()
      if pv == 1:
        for cp in second:
          cp.start()
      ln(0)
      first[1].wait()
      first[2].wait()
      if pv == 2:
        for cp in second:
          cp.start()
      wvt_ref[...] = wqkv_ref[:, 2 * D:3 * D].astype(f32).T.astype(bf16)
      proj(0)
      for cp in second:
        cp.wait()
      for cp in late:
        cp.start()
      ln(1)
      for c in range(1, nx):
        if c + 1 < nx:
          ln(c + 1)
        if c == 1:
          wqt_ref[...] = wqkv_ref[:, 0:D].astype(f32).T.astype(bf16)
        proj(c)
      if early:
        for cp in late:
          cp.wait()

    rows = pl.ds(pl.multiple_of(i * bq, bq), bq)
    qt = lax.dot_general(wqt_ref[...], xn_ref[rows, :], NT, preferred_element_type=f32) * QSCALE
    qtb = qt.astype(bf16)
    for h in range(H):
      qt_ref[h, (h % 8) * DH:(h % 8 + 1) * DH, :] = qtb[h * DH:(h + 1) * DH, :]

    def qmask(h):
      return qt_ref[h]

    def sc_chunk(h, qm, slot, c, m8):
      s = jnp.dot(k_ref[h // 8, c * ck:(c + 1) * ck, :], qm, preferred_element_type=f32)
      s_ref[slot, c * ck:(c + 1) * ck, :] = s
      if mseq:
        s3 = s.reshape(ck // 8, 8, bq)
        for j in range(ck // 8):
          m8 = s3[j] if m8 is None else jnp.maximum(m8, s3[j])
        return m8
      mm = jnp.max(s.reshape(ck // 8, 8, bq), axis=0)
      return mm if m8 is None else jnp.maximum(m8, mm)

    def pv_chunk(h, slot, c, m, l8, o, th=None):
      s3 = s_ref[slot, c * ck:(c + 1) * ck, :].reshape(ck // 8, 8, bq)
      z = l8 if dep else None
      if th is not None:
        z = th if z is None else z + th
      if z is not None:
        m = m + z * 0.0
      p3 = jnp.exp2(s3 - m)
      if seq:
        acc = l8
        for j in range(0, ck // 8, seq):
          t = p3[j]
          for jj in range(1, seq):
            t = t + p3[j + jj]
          acc = t if acc is None else acc + t
        oo = jnp.dot(vt_ref[c * ck // XC, h, :, c * ck % XC:c * ck % XC + ck], p3.reshape(ck, bq).astype(bf16), preferred_element_type=f32)
        return acc, (oo if o is None else o + oo)
      ll = jnp.sum(p3, axis=0)
      oo = jnp.dot(vt_ref[c * ck // XC, h, :, c * ck % XC:c * ck % XC + ck], p3.reshape(ck, bq).astype(bf16), preferred_element_type=f32)
      return (ll, oo) if l8 is None else (l8 + ll, o + oo)

    def gate_up(j, fw):
      xb = xn_ref[rows, :]
      cols = slice(j * fw, (j + 1) * fw)
      g_ = jnp.dot(xb, wg_ref[:, cols], preferred_element_type=f32)
      u_ = jnp.dot(xb, wu_ref[:, cols], preferred_element_type=f32)
      a_ref[:, cols] = (g_ * jax.nn.sigmoid(g_) * u_).astype(bf16)

    def step(h, m, slot, last=False):
      m8 = l8 = o = None
      mh = []
      if c8:
        m = jnp.max(m, axis=0, keepdims=True)
      if not last:
        qm = qmask(h + 1)
      for c in range(nck):
        if not last:
          if order == 0:
            m8 = sc_chunk(h + 1, qm, 1 - slot, c, m8)
            mh.append(m8)
          elif c < nck // order:
            for cc in range(order):
              m8 = sc_chunk(h + 1, qm, 1 - slot, c * order + cc, m8)
        elif fi and c % (nck // 8) == 0 and c // (nck // 8) < 7:
          gate_up(c // (nck // 8), 256)
        l8, o = pv_chunk(h, slot, c, m, l8, o, mh[-1 - sd] if 0 <= sd < len(mh) else None)
      ot_ref[pl.ds(pl.multiple_of(h * DH, DH), DH), :] = o * (1.0 / jnp.sum(l8, axis=0, keepdims=True))
      return None if last else (m8 if c8 else jnp.max(m8, axis=0, keepdims=True))

    qm = qmask(0)
    m8 = None
    for c in range(nck):
      m8 = sc_chunk(0, qm, 0, c, m8)
    m = m8 if c8 else jnp.max(m8, axis=0, keepdims=True)

    def body(j, m):
      for u in range(U):
        m = step(U * j + u, m, u % 2)
      return m
    nit = (H - 1) // U
    m = lax.fori_loop(0, nit, body, m)
    for h in range(nit * U, H - 1):
      m = step(h, m, h % 2)

    if not early:
      @pl.when(i == 0)
      def _():
        for cp in late:
          cp.wait()
    step(H - 1, m, 1, last=True)
    if rb:
      ob_ref[...] = ot_ref[...].T.astype(bf16)
      def ffn_rows(j, carry):
        r = pl.ds(pl.multiple_of(j * rb, rb), rb)
        gr = pl.ds(pl.multiple_of(i * bq + j * rb, rb), rb)
        if fi:
          a = a_ref[r, :]
        else:
          xb = xn_ref[gr, :]
          g_ = jnp.dot(xb, wg_ref[...], preferred_element_type=f32)
          u_ = jnp.dot(xb, wu_ref[...], preferred_element_type=f32)
          a = (g_ * jax.nn.sigmoid(g_) * u_).astype(bf16)
        ffn = jnp.dot(a, wd_ref[...], preferred_element_type=f32)
        attn = jnp.dot(ob_ref[r, :], wo_ref[...], preferred_element_type=f32)
        o_ref[r, :] = (x_ref[gr, :].astype(f32) + attn + ffn).astype(o_ref.dtype)
        return carry
      lax.fori_loop(0, bq // rb, ffn_rows, 0)
    else:
      if not fi:
        gate_up(0, F)
      ffn = jnp.dot(a_ref[...], wd_ref[...], preferred_element_type=f32)
      attn = jnp.dot(ot_ref[...].T.astype(bf16), wo_ref[...], preferred_element_type=f32)
      o_ref[...] = (x_ref[rows, :].astype(f32) + attn + ffn).astype(o_ref.dtype)

  hbm = pl.BlockSpec(memory_space=pl.ANY)
  V = pltpu.VMEM

  @jax.jit
  def run(A_x, A_wqkv, A_wo, B_x, B_w_gate, B_w_up, B_w_down):
    out = pl.pallas_call(
        kern, grid=(S // bq,),
        in_specs=[hbm] * 6,
        out_specs=pl.BlockSpec((bq, D), lambda i: (i, 0)),
        out_shape=jax.ShapeDtypeStruct((S, D), A_x.dtype),
        scratch_shapes=[V((S, D), bf16), V((D, 3 * D), bf16), V((D, D), bf16), V((D, F), bf16), V((D, F), bf16),
                        V((F, D), bf16), pltpu.SemaphoreType.DMA((S // XC + 7,)),
                        V((S, D), bf16), V((4, S, 128), bf16), V((S // XC, H, DH, XC), bf16), V((D, D), bf16),
                        V((H, 128, bq), bf16), V((D, bq), f32), V((2, S, bq), f32), V((bq, F), bf16), V((D, D), bf16), V((bq, D), bf16)],
        compiler_params=pltpu.CompilerParams(dimension_semantics=("arbitrary",), vmem_limit_bytes=100 * 2**20, flags=flags),
    )(A_x.reshape(S, D), A_wqkv, A_wo, B_w_gate, B_w_up, B_w_down)
    return out.reshape(1, S, D)
  return run


_run = make(XC=512, pv=1)


@jax.jit
def pallas_parallel_sum__mha_block__swiglu_ffn__prompt_kernel(A_x, A_wqkv, A_wo, B_x, B_w_gate, B_w_up, B_w_down):
  return _run(A_x, A_wqkv, A_wo, B_x, B_w_gate, B_w_up, B_w_down)
```

```python
import jax
import jax.numpy as jnp
import numpy as np
from jax import lax
import jax.experimental.pallas as pl
import jax.experimental.pallas.tpu as pltpu

S, D, H, DH, F = 2048, 512, 32, 16, 1792
f32, bf16 = jnp.float32, jnp.bfloat16
QSCALE = float(DH ** -0.5 * np.log2(np.e))
NT = (((1,), (1,)), ((), ()))
XC_ = 256


def make(bq=512, ck=128, U=2, dep=1, fi=1, rb=0, XC=256, order=0, c8=1, xh=1, pv=0, seq=0, mseq=0, early=1, sd=-1, flags=None):
  nck = S // ck

  def kern(x_hbm, wqkv_hbm, wo_hbm, wg_hbm, wu_hbm, wd_hbm, o_ref,
           x_ref, wqkv_ref, wo_ref, wg_ref, wu_ref, wd_ref, sems,
           xn_ref, k_ref, vt_ref, wqt_ref, qt_ref, ot_ref, s_ref, a_ref, wvt_ref, ob_ref):
    i = pl.program_id(0)
    nx = S // XC

    def x_copy(c):
      r = pl.ds(c * XC, XC)
      return pltpu.make_async_copy(x_hbm.at[r, :], x_ref.at[r, :], sems.at[c])
    def w_copy(j):
      cols = pl.ds(j * D, D)
      return pltpu.make_async_copy(wqkv_hbm.at[:, cols], wqkv_ref.at[:, cols], sems.at[nx + j])
    late = [pltpu.make_async_copy(a, b, sems.at[nx + 3 + j]) for j, (a, b) in enumerate(
        ((wg_hbm, wg_ref), (wu_hbm, wu_ref), (wd_hbm, wd_ref), (wo_hbm, wo_ref)))]

    @pl.when(i == 0)
    def _():
      def ln(c):
        r = slice(c * XC, (c + 1) * XC)
        x = x_ref[r, :].astype(f32)
        xc = x - jnp.mean(x, axis=-1, keepdims=True)
        v = jnp.mean(xc * xc, axis=-1, keepdims=True)
        xn_ref[r, :] = (xc * lax.rsqrt(v + 1e-5)).astype(bf16)
      def proj(c):
        r = slice(c * XC, (c + 1) * XC)
        xn = xn_ref[r, :]
        kk = jnp.dot(xn, wqkv_ref[:, D:2 * D], preferred_element_type=f32).astype(bf16)
        for g in range(4):
          k_ref[g, r, :] = kk[:, g * 128:(g + 1) * 128]
        vt_ref[c] = lax.dot_general(wvt_ref[...], xn, NT, preferred_element_type=f32).astype(bf16).reshape(H, DH, XC)
      first = [x_copy(0), w_copy(1), w_copy(2)]
      second = [x_copy(c) for c in range(1, nx)] + [w_copy(0)]
      if pv == 0:
        for cp in first + second:
          cp.start()
      else:
        for cp in first:
          cp.start()
      qt_ref[...] = jnp.zeros(qt_ref.shape, bf16)
      first[0].wait()
      if pv == 1:
        for cp in second:
          cp.start()
      ln(0)
      first[1].wait()
      first[2].wait()
      if pv == 2:
        for cp in second:
          cp.start()
      wvt_ref[...] = wqkv_ref[:, 2 * D:3 * D].astype(f32).T.astype(bf16)
      proj(0)
      for cp in second:
        cp.wait()
      for cp in late:
        cp.start()
      ln(1)
      for c in range(1, nx):
        if c + 1 < nx:
          ln(c + 1)
        if c == 1:
          wqt_ref[...] = wqkv_ref[:, 0:D].astype(f32).T.astype(bf16)
        proj(c)
      if early:
        for cp in late:
          cp.wait()

    rows = pl.ds(pl.multiple_of(i * bq, bq), bq)
    qt = lax.dot_general(wqt_ref[...], xn_ref[rows, :], NT, preferred_element_type=f32) * QSCALE
    qtb = qt.astype(bf16)
    for h in range(H):
      qt_ref[h, (h % 8) * DH:(h % 8 + 1) * DH, :] = qtb[h * DH:(h + 1) * DH, :]

    def qmask(h):
      return qt_ref[h]

    prev = [None]

    def sc_chunk(h, qm, slot, c, m8):
      s = jnp.dot(k_ref[h // 8, c * ck:(c + 1) * ck, :], qm, preferred_element_type=f32)
      s_ref[slot, c * ck:(c + 1) * ck, :] = s
      if mseq:
        s3 = s.reshape(ck // 8, 8, bq)
        for j in range(ck // 8):
          m8 = s3[j] if m8 is None else jnp.maximum(m8, s3[j])
        return m8
      mm = jnp.max(s.reshape(ck // 8, 8, bq), axis=0)
      return mm if m8 is None else jnp.maximum(m8, mm)

    def pv_chunk(h, slot, c, m, l8, o, th=None):
      s3 = s_ref[slot, c * ck:(c + 1) * ck, :].reshape(ck // 8, 8, bq)
      z = l8 if dep else None
      if th is not None:
        z = th if z is None else z + th
      if z is not None:
        m = m + z * 0.0
      p3 = jnp.exp2(s3 - m)
      if seq:
        acc = l8
        for j in range(0, ck // 8, seq):
          t = p3[j]
          for jj in range(1, seq):
            t = t + p3[j + jj]
          acc = t if acc is None else acc + t
        oo = jnp.dot(vt_ref[c * ck // XC, h, :, c * ck % XC:c * ck % XC + ck], p3.reshape(ck, bq).astype(bf16), preferred_element_type=f32)
        return acc, (oo if o is None else o + oo)
      ll = jnp.sum(p3, axis=0)
      oo = jnp.dot(vt_ref[c * ck // XC, h, :, c * ck % XC:c * ck % XC + ck], p3.reshape(ck, bq).astype(bf16), preferred_element_type=f32)
      return (ll, oo) if l8 is None else (l8 + ll, o + oo)

    def gate_up(j, fw):
      xb = xn_ref[rows, :]
      cols = slice(j * fw, (j + 1) * fw)
      g_ = jnp.dot(xb, wg_ref[:, cols], preferred_element_type=f32)
      u_ = jnp.dot(xb, wu_ref[:, cols], preferred_element_type=f32)
      a_ref[:, cols] = (g_ * jax.nn.sigmoid(g_) * u_).astype(bf16)

    def step(h, m, slot, last=False):
      m8 = l8 = o = None
      mh = []
      if c8:
        m = jnp.max(m, axis=0, keepdims=True)
      if not last:
        qm = qmask(h + 1)
      for c in range(nck):
        if not last:
          if order == 0:
            m8 = sc_chunk(h + 1, qm, 1 - slot, c, m8)
            mh.append(m8)
          elif c < nck // order:
            for cc in range(order):
              m8 = sc_chunk(h + 1, qm, 1 - slot, c * order + cc, m8)
        elif fi and c % (nck // 8) == 0 and c // (nck // 8) < 7:
          gate_up(c // (nck // 8), 256)
        l8, o = pv_chunk(h, slot, c, m, l8, o, prev[0] if (xh and c == 0) else None)
      ot_ref[pl.ds(pl.multiple_of(h * DH, DH), DH), :] = o * (1.0 / jnp.sum(l8, axis=0, keepdims=True))
      prev[0] = l8
      return None if last else (m8 if c8 else jnp.max(m8, axis=0, keepdims=True))

    qm = qmask(0)
    m8 = None
    for c in range(nck):
      m8 = sc_chunk(0, qm, 0, c, m8)
    m = m8 if c8 else jnp.max(m8, axis=0, keepdims=True)

    def body(j, m):
      for u in range(U):
        m = step(U * j + u, m, u % 2)
      prev[0] = None
      return m
    nit = (H - 1) // U
    m = lax.fori_loop(0, nit, body, m)
    for h in range(nit * U, H - 1):
      m = step(h, m, h % 2)

    if not early:
      @pl.when(i == 0)
      def _():
        for cp in late:
          cp.wait()
    step(H - 1, m, 1, last=True)
    if rb:
      ob_ref[...] = ot_ref[...].T.astype(bf16)
      def ffn_rows(j, carry):
        r = pl.ds(pl.multiple_of(j * rb, rb), rb)
        gr = pl.ds(pl.multiple_of(i * bq + j * rb, rb), rb)
        if fi:
          a = a_ref[r, :]
        else:
          xb = xn_ref[gr, :]
          g_ = jnp.dot(xb, wg_ref[...], preferred_element_type=f32)
          u_ = jnp.dot(xb, wu_ref[...], preferred_element_type=f32)
          a = (g_ * jax.nn.sigmoid(g_) * u_).astype(bf16)
        ffn = jnp.dot(a, wd_ref[...], preferred_element_type=f32)
        attn = jnp.dot(ob_ref[r, :], wo_ref[...], preferred_element_type=f32)
        o_ref[r, :] = (x_ref[gr, :].astype(f32) + attn + ffn).astype(o_ref.dtype)
        return carry
      lax.fori_loop(0, bq // rb, ffn_rows, 0)
    else:
      if not fi:
        gate_up(0, F)
      ffn = jnp.dot(a_ref[...], wd_ref[...], preferred_element_type=f32)
      attn = jnp.dot(ot_ref[...].T.astype(bf16), wo_ref[...], preferred_element_type=f32)
      o_ref[...] = (x_ref[rows, :].astype(f32) + attn + ffn).astype(o_ref.dtype)

  hbm = pl.BlockSpec(memory_space=pl.ANY)
  V = pltpu.VMEM

  @jax.jit
  def run(A_x, A_wqkv, A_wo, B_x, B_w_gate, B_w_up, B_w_down):
    out = pl.pallas_call(
        kern, grid=(S // bq,),
        in_specs=[hbm] * 6,
        out_specs=pl.BlockSpec((bq, D), lambda i: (i, 0)),
        out_shape=jax.ShapeDtypeStruct((S, D), A_x.dtype),
        scratch_shapes=[V((S, D), bf16), V((D, 3 * D), bf16), V((D, D), bf16), V((D, F), bf16), V((D, F), bf16),
                        V((F, D), bf16), pltpu.SemaphoreType.DMA((S // XC + 7,)),
                        V((S, D), bf16), V((4, S, 128), bf16), V((S // XC, H, DH, XC), bf16), V((D, D), bf16),
                        V((H, 128, bq), bf16), V((D, bq), f32), V((2, S, bq), f32), V((bq, F), bf16), V((D, D), bf16), V((bq, D), bf16)],
        compiler_params=pltpu.CompilerParams(dimension_semantics=("arbitrary",), vmem_limit_bytes=100 * 2**20, flags=flags),
    )(A_x.reshape(S, D), A_wqkv, A_wo, B_w_gate, B_w_up, B_w_down)
    return out.reshape(1, S, D)
  return run


_run = make(XC=512, pv=1, seq=1)


@jax.jit
def pallas_parallel_sum__mha_block__swiglu_ffn__prompt_kernel(A_x, A_wqkv, A_wo, B_x, B_w_gate, B_w_up, B_w_down):
  return _run(A_x, A_wqkv, A_wo, B_x, B_w_gate, B_w_up, B_w_down)
```
